```python
import os as _os
_os.environ.setdefault("JAX_PLATFORMS", "cpu")
import jax
import jax.numpy as jnp

def _softmax(x, axis=-1):
    return jax.nn.softmax(x, axis=axis)
def _gelu(x):
    return jax.nn.gelu(x, approximate=True)
def _silu(x):
    return jax.nn.silu(x)
def _sigmoid(x):
    return jax.nn.sigmoid(x)
def _layernorm(x, axis=-1, eps=1e-5):
    m = jnp.mean(x, axis=axis, keepdims=True)
    v = jnp.var(x, axis=axis, keepdims=True)
    return (x - m) / jnp.sqrt(v + eps)
def _scatter_add(tgt, idx, src, axis=0):
    return tgt.at[idx].add(src)
def _segment_sum(src, seg, n):
    return jax.ops.segment_sum(src, seg, n)
class _Rng:
    def __init__(self, key):
        self._k = key
    def _next(self):
        self._k, sub = jax.random.split(self._k)
        return sub
    def normal(self, shape):
        return jax.random.normal(self._next(), shape, dtype=jnp.bfloat16)
    def randint(self, lo, hi, shape):
        return jax.random.randint(self._next(), shape, lo, hi, dtype=jnp.int32)
    def uniform(self, shape, lo=0.0, hi=1.0):
        return jax.random.uniform(self._next(), shape, jnp.bfloat16, lo, hi)
    def permutation(self, n):
        return jax.random.permutation(self._next(), n)


kernel_name = 'concat_heads__sliding_block__grouped_kv_mqa__prompt'

def setup_inputs():
    _rng = _Rng(jax.random.key(int.from_bytes(__import__("os").urandom(4), "little")))
    _w = (lambda a: (lambda t: t.astype(jnp.bfloat16) if jnp.issubdtype(t.dtype, jnp.floating) else t)(jnp.asarray(a)))
    def _A_setup():
        B, S, D = 1, 2048, 576
        return {
            "x": _w((lambda *s: _rng.normal(s) * 0.2)(B, S, D)),
            "wqkv": _w((lambda *s: _rng.normal(s) * 0.2)(D, 3 * D)),
            "wo": _w((lambda *s: _rng.normal(s) * 0.05)(D, D)),
        }
    _A_in = _A_setup()

    def _B_setup():
        B, S, D, H = 1, 2048, 576, 32
        Dh = D // H
        return {
            "x": _w((lambda *s: _rng.normal(s) * 0.05)(B, S, D)),
            "wq": _w((lambda *s: _rng.normal(s) * 1.6)(D, H * Dh)),
            "wk": _w((lambda *s: _rng.normal(s) * 1.6)(D, Dh)),
            "wv": _w((lambda *s: _rng.normal(s) * 0.1)(D, Dh)),
            "wo": _w((lambda *s: _rng.normal(s) * 0.1)(H * Dh, D)),
        }
    _B_in = _B_setup()

    return {
        "A_x": _A_in["x"],
        "A_wqkv": _A_in["wqkv"],
        "A_wo": _A_in["wo"],
        "B_x": _B_in["x"],
        "B_wq": _B_in["wq"],
        "B_wk": _B_in["wk"],
        "B_wv": _B_in["wv"],
        "B_wo": _B_in["wo"],
    }

def reference(A_x, A_wqkv, A_wo, B_x, B_wq, B_wk, B_wv, B_wo):
    def _A_ref(x, wqkv, wo):
        B, S, D = x.shape
        H = 32; Dh = D // H; W = 256
        qkv = (lambda x, *d: x.transpose(*d))((x @ wqkv).reshape(B, S, 3, H, Dh), 2, 0, 3, 1, 4)
        q, k, v = qkv[0], qkv[1], qkv[2]
        scores = jnp.einsum("bhqd,bhkd->bhqk", q, k) * (Dh ** -0.5)
        idx = jnp.arange(S)
        mask = (idx[:, None] - idx[None, :] >= 0) & (idx[:, None] - idx[None, :] < W)
        scores = jnp.where(mask[None, None], scores, -1e9)
        p = _softmax(scores, axis=-1)
        o = jnp.einsum("bhqk,bhkd->bhqd", p, v)
        return (lambda x, *d: x.transpose(*d))(o, 0, 2, 1, 3).reshape(B, S, D) @ wo

    def _B_ref(x, wq, wk, wv, wo):
        B, S, D = x.shape
        H = 32
        Dh = D // H
        q = (lambda x, *d: x.transpose(*d))((x @ wq).reshape(B, S, H, Dh), 0, 2, 1, 3)
        k = x @ wk
        v = x @ wv
        scores = jnp.einsum("bhqd,bkd->bhqk", q, k) * (Dh ** -0.5)
        p = _softmax(scores, axis=-1)
        o = jnp.einsum("bhqk,bkd->bhqd", p, v)
        return (lambda x, *d: x.transpose(*d))(o, 0, 2, 1, 3).reshape(B, S, H * Dh) @ wo

    a = _A_ref(A_x, A_wqkv, A_wo)
    b = _B_ref(B_x, B_wq, B_wk, B_wv, B_wo)
    return jnp.concatenate([a, b], axis=-1)
```

```python
import functools
import math

import jax
import jax.numpy as jnp
from jax import lax
import jax.experimental.pallas as pl
import jax.experimental.pallas.tpu as pltpu

S = 2048
D = 576
H = 32
DH = 18
HG = 7
NG = 5
GW = HG * DH
VR = 24
PADK = 256
NB_ = 512
TC = 512
NTC = S // TC
NEG = -1e30
SCALE = float(DH ** -0.5) * math.log2(math.e)
F32 = jnp.float32
BF16 = jnp.bfloat16

TN = (((0,), (0,)), ((), ()))


def _dot(a, b):
    return jnp.dot(a, b, preferred_element_type=F32)


def _dg(a, b, dn):
    return lax.dot_general(a, b, dn, preferred_element_type=F32)


def _group_cols(w, off):
    parts = []
    for g in range(NG):
        lo = off + GW * g
        if g < NG - 1:
            parts.append(w[:, lo:lo + 128])
        else:
            n = D - GW * g
            parts.append(w[:, lo:lo + n])
            parts.append(jnp.zeros((w.shape[0], 128 - n), w.dtype))
    return jnp.concatenate(parts, axis=1)


def _kernel(xa_hbm, wqkv_hbm, woa_hbm, xb_hbm, wq_hbm, wk_hbm, wv_hbm, wob_hbm, out_hbm,
            xa, xb, wqkv, woa, wob, wq, wk, wv, obuf, isem, osem,
            wta, wka, wtb, qa, ka, vta, qb, kb, vtb, sa, sb, ma, mb, ota, otb):
    def cp(i, src, dst):
        return pltpu.make_async_copy(src, dst, isem.at[i])

    def xs(ref, t):
        return ref.at[:, pl.ds(t * TC, TC)]

    first = [cp(0, wk_hbm, wk), cp(1, wv_hbm, wv), cp(2, wq_hbm, wq), cp(3, xs(xb_hbm, 0), xs(xb, 0))]
    rest_b = [cp(3 + t, xs(xb_hbm, t), xs(xb, t)) for t in range(1, NTC)]
    w_a = cp(3 + NTC, wqkv_hbm, wqkv)
    x_a = [cp(4 + NTC + t, xs(xa_hbm, t), xs(xa, t)) for t in range(NTC)]
    w_o = [cp(4 + 2 * NTC, woa_hbm, woa), cp(5 + 2 * NTC, wob_hbm, wob)]
    for c in first:
        c.start()
    for g in range(NG):
        ka[g, 0:PADK, :] = jnp.zeros((PADK, 128), BF16)
    vta[:, 0:PADK] = jnp.zeros((D, PADK), F32)
    for c in first:
        c.wait()
    for c in rest_b + [w_a] + x_a + w_o:
        c.start()

    wtb[0:NG * 128, :] = _group_cols(wq[...], 0).T
    wkf = wk[...].astype(F32)
    wtb[NG * 128:NG * 128 + 128, :] = jnp.concatenate(
        [wkf] * HG + [jnp.zeros((128 - GW, D), F32)], axis=0).astype(BF16)
    wtb[NG * 128 + 128:, :] = jnp.concatenate(
        [wv[...].astype(F32), jnp.zeros((32 - DH, D), F32)], axis=0).astype(BF16)
    rowv = lax.broadcasted_iota(jnp.int32, (VR, TC), 0)
    for t in range(NTC):
        if t > 0:
            rest_b[t - 1].wait()
        ts = slice(t * TC, (t + 1) * TC)
        r = _dot(wtb[...], xb[:, ts])
        qb[:, ts] = (r[0:NG * 128] * SCALE).astype(BF16)
        kb[ts, :] = r[NG * 128:NG * 128 + 128].T.astype(BF16)
        vtb0 = r[NG * 128 + 128:NG * 128 + 128 + VR].astype(BF16).astype(F32)
        vtb0 = jnp.where(rowv == DH, 1.0, vtb0)
        for i in range(4):
            vtb[i, :, ts] = vtb0 if i == 0 else pltpu.roll(vtb0, 2 * i, 0)

    w_a.wait()
    w = wqkv[...]
    wta[0:NG * 128, :] = _group_cols(w, 0).T
    wka[...] = _group_cols(w, D)
    wta[NG * 128:, :] = w[:, 2 * D:3 * D].T
    for t in range(NTC):
        x_a[t].wait()
        ts = slice(t * TC, (t + 1) * TC)
        tp = slice(PADK + t * TC, PADK + (t + 1) * TC)
        xc = xa[:, ts]
        r = _dot(wta[...], xc)
        qa[:, ts] = (r[0:NG * 128] * SCALE).astype(BF16)
        vta[:, tp] = r[NG * 128:].astype(BF16).astype(F32)
        kk = _dg(xc, wka[...], TN)
        for g in range(NG):
            ka[g, tp, :] = kk[:, g * 128:(g + 1) * 128].astype(BF16)

    r128 = lax.broadcasted_iota(jnp.int32, (128, 128), 0)
    c128 = lax.broadcasted_iota(jnp.int32, (128, 128), 1)
    rvr = lax.broadcasted_iota(jnp.int32, (VR, 128), 0)
    rvr_b = lax.broadcasted_iota(jnp.int32, (VR, NB_), 0)

    def mask_q(q, j):
        qi = pltpu.bitcast(q, jnp.int32)
        row = lax.broadcasted_iota(jnp.int32, qi.shape, 0)
        qi = jnp.where((row >= (DH // 2) * j) & (row < (DH // 2) * (j + 1)), qi, 0)
        return pltpu.bitcast(qi, BF16)

    def step(h, do_qk, do_pv):
        if do_qk:
            h1 = h + 1
            g1 = h1 // HG
            j1 = h1 - g1 * HG
            r1 = pl.multiple_of(g1 * 128, 128)
        if do_pv:
            o = (h * DH) & 7
            w0 = pl.multiple_of(h * DH - o, 8)
            one_pos = jnp.where(o == 6, 0, o + DH)
            vi = o >> 1
        for n in range(S // NB_):
            cs = slice(n * NB_, (n + 1) * NB_)
            if do_qk:
                qm = mask_q(qb[pl.ds(r1, 128), cs], j1)
            if do_pv:
                m_cur = mb[:, cs]
            acc = None
            mx = None
            for c in range(S // 128):
                ks = slice(c * 128, (c + 1) * 128)
                if do_pv:
                    p = jnp.exp2(sb[ks, cs] - m_cur).astype(BF16)
                    d = _dot(vtb[vi, :, ks], p)
                    acc = d if acc is None else acc + d
                if do_qk:
                    s = _dot(kb[ks, :], qm)
                    sb[ks, cs] = s
                    mc = jnp.max(s.reshape(16, 8, NB_), axis=0)
                    mx = mc if mx is None else jnp.maximum(mx, mc)
                if c == 3 and do_pv:
                    m_a = ma[:, cs]
                    p1 = jnp.exp2(sa[0:128, cs] - m_a).astype(BF16)
                    pm = jnp.exp2(sa[128:256, cs] - m_a)
                    accs = []
                    for uu in range(4):
                        u = n * 4 + uu
                        us = slice(uu * 128, (uu + 1) * 128)
                        p0 = jnp.where(r128 > c128, pm[:, us], 0.0).astype(BF16)
                        p2 = jnp.where(r128 > c128, 0.0, pm[:, us]).astype(BF16)
                        acca = None
                        for t, pt in ((0, p0), (1, p1[:, us]), (2, p2)):
                            if u + t < 2:
                                continue
                            vt = vta[pl.ds(w0, VR), (u + t) * 128:(u + t + 1) * 128]
                            vt = jnp.where(rvr == one_pos, 1.0, vt)
                            d = _dot(vt, pt)
                            acca = d if acca is None else acca + d
                        accs.append(acca)
                    acca = jnp.concatenate(accs, axis=1)
                    l = jnp.sum(jnp.where(rvr_b == one_pos, acca, 0.0), axis=0, keepdims=True)
                    pltpu.store(ota.at[pl.ds(w0, VR), cs], acca * (1.0 / l),
                                mask=(rvr_b >= o) & (rvr_b < o + DH))
                if c == 9 and do_qk:
                    qma = mask_q(qa[pl.ds(r1, 128), cs], j1)
                    ms = []
                    for uu in range(4):
                        u = n * 4 + uu
                        us = slice(uu * 128, (uu + 1) * 128)
                        ug = slice(u * 128, (u + 1) * 128)
                        if u >= 2:
                            s3 = _dot(ka[g1, u * 128:(u + 3) * 128, :], qma[:, us])
                            s1 = s3[128:256]
                            sm = jnp.where(r128 > c128, s3[0:128], s3[256:384])
                        elif u == 1:
                            s3 = _dot(ka[g1, (u + 1) * 128:(u + 3) * 128, :], qma[:, us])
                            s1 = s3[0:128]
                            sm = jnp.where(r128 > c128, NEG, s3[128:256])
                        else:
                            s3 = _dot(ka[g1, (u + 2) * 128:(u + 3) * 128, :], qma[:, us])
                            s1 = jnp.full((128, 128), NEG, F32)
                            sm = jnp.where(r128 > c128, NEG, s3)
                        sa[0:128, ug] = s1
                        sa[128:256, ug] = sm
                        ms.append(jnp.max(jnp.maximum(s1, sm), axis=0, keepdims=True))
                    ma[:, cs] = jnp.concatenate(ms, axis=1)
            if do_pv:
                l = jnp.sum(jnp.where(rvr_b == one_pos, acc, 0.0), axis=0, keepdims=True)
                pltpu.store(otb.at[pl.ds(w0, VR), cs], acc * (1.0 / l),
                            mask=(rvr_b >= o) & (rvr_b < o + DH))
            if do_qk:
                mb[:, cs] = jnp.max(mx, axis=0, keepdims=True)

    step(-1, True, False)

    def body(h, c):
        step(h, True, True)
        return c

    lax.fori_loop(0, H - 1, body, 0)
    step(H - 1, False, True)

    for c in w_o:
        c.wait()
    outs = []
    for t in range(NTC):
        ts = slice(t * TC, (t + 1) * TC)
        oa = ota[:, ts].astype(BF16)
        ob = otb[:, ts].astype(BF16)
        ya = _dg(oa, woa[...], TN)
        yb = _dg(ob, wob[...], TN)
        obuf[t] = jnp.concatenate([ya, yb], axis=1).astype(BF16)
        c = pltpu.make_async_copy(obuf.at[t], out_hbm.at[pl.ds(t * TC, TC), :], osem.at[t])
        c.start()
        outs.append(c)
    for c in outs:
        c.wait()


@jax.jit
def pallas_concat_heads__sliding_block__grouped_kv_mqa__prompt_kernel(
    A_x, A_wqkv, A_wo, B_x, B_wq, B_wk, B_wv, B_wo,
):
    hbm = pl.BlockSpec(memory_space=pl.ANY)
    out = pl.pallas_call(
        _kernel,
        out_shape=jax.ShapeDtypeStruct((S, 2 * D), BF16),
        in_specs=[hbm] * 8,
        out_specs=hbm,
        scratch_shapes=[
            pltpu.VMEM((D, S), BF16),
            pltpu.VMEM((D, S), BF16),
            pltpu.VMEM((D, 3 * D), BF16),
            pltpu.VMEM((D, D), BF16),
            pltpu.VMEM((D, D), BF16),
            pltpu.VMEM((D, D), BF16),
            pltpu.VMEM((DH, D), BF16),
            pltpu.VMEM((DH, D), BF16),
            pltpu.VMEM((NTC, TC, 2 * D), BF16),
            pltpu.SemaphoreType.DMA((6 + 2 * NTC,)),
            pltpu.SemaphoreType.DMA((NTC,)),
            pltpu.VMEM((NG * 128 + D, D), BF16),
            pltpu.VMEM((D, NG * 128), BF16),
            pltpu.VMEM((NG * 128 + 128 + 32, D), BF16),
            pltpu.VMEM((NG * 128, S), BF16),
            pltpu.VMEM((NG, S + PADK, 128), BF16),
            pltpu.VMEM((D, S + PADK), F32),
            pltpu.VMEM((NG * 128, S), BF16),
            pltpu.VMEM((S, 128), BF16),
            pltpu.VMEM((4, VR, S), F32),
            pltpu.VMEM((256, S), F32),
            pltpu.VMEM((S, S), F32),
            pltpu.VMEM((1, S), F32),
            pltpu.VMEM((1, S), F32),
            pltpu.VMEM((D, S), F32),
            pltpu.VMEM((D, S), F32),
        ],
        compiler_params=pltpu.CompilerParams(vmem_limit_bytes=120 * 1024 * 1024),
        name="fused_attn",
    )(A_x.reshape(S, D).T, A_wqkv, A_wo, B_x.reshape(S, D).T, B_wq, B_wk.T, B_wv.T, B_wo)
    return out.reshape(1, S, 2 * D)
```

```python
import math

import jax
import jax.numpy as jnp
from jax import lax
import jax.experimental.pallas as pl
import jax.experimental.pallas.tpu as pltpu

S = 2048
D = 576
H = 32
DH = 18
HG = 7
NG = 5
GW = HG * DH
VR = 24
PADK = 256
NB = 512
NCH = S // 128
TC = 512
NTC = S // TC
KVR = 48
CP1, CP0, CQA = 1, 4, 9
NEG = -1e30
SCALE = float(DH ** -0.5) * math.log2(math.e)
F32 = jnp.float32
BF16 = jnp.bfloat16
I32 = jnp.int32

TN = (((0,), (0,)), ((), ()))


def _dot(a, b):
    return jnp.dot(a, b, preferred_element_type=F32)


def _dot_tn(a, b):
    return lax.dot_general(a, b, TN, preferred_element_type=F32)


def _bf16_rows(x_i32):
    return pltpu.bitcast(x_i32, BF16)


def _pack_rows(x_bf16):
    return pltpu.bitcast(x_bf16, I32)


def _kernel(xa_hbm, wqkv_hbm, woa_hbm, xb_hbm, wq_hbm, wk_hbm, wv_hbm, wob_hbm, out_hbm,
            xa, xb, wqkv, woa, wob, wq, wk, wv, obuf, isem, xsem, osem,
            wkv, qa, ka, vta, qb, kb, vtb, sa, sb, ma, mb, ota, otb):
    def cp(i, src, dst):
        return pltpu.make_async_copy(src, dst, isem.at[i])

    def xcp(b, t):
        src, dst = ((xb_hbm, xb), (xa_hbm, xa))[b]
        ts = pl.ds(pl.multiple_of(t * TC, TC), TC)
        return pltpu.make_async_copy(src.at[:, ts], dst.at[:, ts], xsem.at[b * NTC + t])

    first = [cp(0, wk_hbm, wk), cp(1, wv_hbm, wv), cp(2, wq_hbm, wq)]
    w_a = cp(3, wqkv_hbm, wqkv)
    w_o = [cp(4, woa_hbm, woa), cp(5, wob_hbm, wob)]
    for c in first:
        c.start()
    xcp(0, 0).start()
    for g in range(NG):
        ka[g, 0:PADK // 2, :] = jnp.zeros((PADK // 2, 128), I32)
    vta[:, 0:PADK] = jnp.zeros((D, PADK), F32)
    for c in first:
        c.wait()
    xcp(0, 1).start()
    xcp(0, 2).start()

    wkv[...] = jnp.concatenate(
        [wk[...].astype(F32), wv[...].astype(F32), jnp.zeros((KVR - 2 * DH, D), F32)],
        axis=0).astype(BF16)
    rowv = lax.broadcasted_iota(I32, (VR, TC), 0)

    def store_q(q_ref, rq, ts):
        for g in range(NG):
            gr = 128 if g < NG - 1 else 80
            qf = rq[g * GW:min(g * GW + gr, rq.shape[0])]
            if qf.shape[0] < gr:
                qf = jnp.concatenate([qf, jnp.zeros((gr - qf.shape[0], TC), F32)], axis=0)
            q_ref[g * 64:g * 64 + gr // 2, ts] = _pack_rows((qf * SCALE).astype(BF16))

    def proj_b(t, carry):
        xcp(0, t).wait()

        @pl.when(t == 0)
        def _():
            xcp(0, 3).start()
            w_a.start()

        @pl.when(t == 1)
        def _():
            xcp(1, 0).start()
            for c in w_o:
                c.start()

        @pl.when(t == 2)
        def _():
            for u in range(1, NTC):
                xcp(1, u).start()

        ts = pl.ds(pl.multiple_of(t * TC, TC), TC)
        r = _dot(wkv[...], xb[:, ts])
        store_q(qb, _dot_tn(wq[...], xb[:, ts]), ts)
        kt = r[0:DH]
        k16 = jnp.concatenate([kt] * HG + [kt[0:128 - GW]], axis=0).astype(BF16).T
        kb[pl.ds(pl.multiple_of(t * (TC // 2), TC // 2), TC // 2), :] = _pack_rows(k16)
        vt = r[DH:DH + VR].astype(BF16).astype(F32)
        vt = jnp.where(rowv == DH, 1.0, jnp.where(rowv < DH, vt, 0.0))
        for i in range(4):
            vtb[i, :, ts] = vt if i == 0 else pltpu.roll(vt, 2 * i, 0)
        return carry

    lax.fori_loop(0, NTC, proj_b, 0)

    w_a.wait()

    def proj_a(t, carry):
        xcp(1, t).wait()
        ts = pl.ds(pl.multiple_of(t * TC, TC), TC)
        tp = pl.ds(pl.multiple_of(PADK + t * TC, TC // 2), TC)
        tp2 = pl.ds(pl.multiple_of((PADK + t * TC) // 2, TC // 4), TC // 2)
        r = _dot_tn(wqkv[...], xa[:, ts])
        store_q(qa, r[0:2 * D], ts)
        for g in range(NG):
            ka[g, tp2, :] = _pack_rows(r[D + g * GW:D + g * GW + 128].astype(BF16).T)
        vta[:, tp] = r[2 * D:].astype(BF16).astype(F32)
        return carry

    lax.fori_loop(0, NTC, proj_a, 0)

    tri = (lax.broadcasted_iota(I32, (128, NB), 0)[:, 0:128]
           > (lax.broadcasted_iota(I32, (128, NB), 1) & 127)[:, 0:128])
    r64 = lax.broadcasted_iota(I32, (64, 128), 0)
    c64 = lax.broadcasted_iota(I32, (64, 128), 1)
    tri_i32 = jnp.where(2 * r64 > c64, 0xFFFF, 0) | jnp.where(2 * r64 + 1 > c64, -65536, 0)
    rvr = lax.broadcasted_iota(I32, (VR, 128), 0)
    rvr_b = lax.broadcasted_iota(I32, (VR, NB), 0)

    def mask_q(qi, j):
        row = lax.broadcasted_iota(I32, qi.shape, 0)
        return _bf16_rows(jnp.where((row >= (DH // 2) * j) & (row < (DH // 2) * (j + 1)), qi, 0))

    def block(h, n, do_qk, do_pv, hook=None, gj=None):
        static_n = isinstance(n, int)
        c0 = n * NB if static_n else pl.multiple_of(n * NB, NB)
        c02 = c0 // 2 if static_n else pl.multiple_of(n * (NB // 2), NB // 2)
        cs = pl.ds(c0, NB)
        if do_qk:
            g1, j1 = gj if gj is not None else divmod(h + 1, HG)
            r1 = g1 * 64 if isinstance(g1, int) else pl.multiple_of(g1 * 64, 64)
            qm = mask_q(qb[pl.ds(r1, 64), cs], j1)
        if do_pv:
            o = (h * DH) & 7
            w0 = h * DH - o
            w0 = w0 if isinstance(h, int) else pl.multiple_of(w0, 8)
            one_pos = jnp.where(o == 6, 0, o + DH) if not isinstance(h, int) else (o + DH) % VR
            vi = o >> 1
            m_cur = mb[:, cs]

        def normalize_store(dst, acc):
            l = jnp.sum(jnp.where(rvr_b == one_pos, acc, 0.0), axis=0, keepdims=True)
            pltpu.store(dst.at[pl.ds(w0, VR), cs], acc * (1.0 / l),
                        mask=(rvr_b >= o) & (rvr_b < o + DH))

        def pv_a(t, pt):
            res = []
            for uu in range(4):
                vt = vta[pl.ds(w0, VR), pl.ds(c0 + (uu + t) * 128, 128)]
                vt = jnp.where(rvr == one_pos, 1.0, vt)
                res.append(_dot(vt, pt[uu]))
            return jnp.concatenate(res, axis=1)

        acc = mx = acca = None
        for c in range(NCH):
            ks = slice(c * 128, (c + 1) * 128)
            if hook is not None:
                hook(c)
            if do_pv:
                p = jnp.exp2(sb[ks, cs] - m_cur).astype(BF16)
                d = _dot(vtb[vi, :, ks], p)
                acc = d if acc is None else acc + d
            if do_qk:
                s = _dot(_bf16_rows(kb[c * 64:(c + 1) * 64, :]), qm)
                sb[ks, cs] = s
                mc = jnp.max(s.reshape(16, 8, NB), axis=0)
                mx = mc if mx is None else jnp.maximum(mx, mc)
            if do_pv:
                if c == CP1:
                    m_a = ma[:, cs]
                    p1 = jnp.exp2(sa[0:128, cs] - m_a)
                    acca = pv_a(1, [p1[:, uu * 128:(uu + 1) * 128].astype(BF16) for uu in range(4)])
                if c == CP0:
                    pm = jnp.exp2(sa[128:256, cs] - m_a)
                    pmi = [_pack_rows(pm[:, uu * 128:(uu + 1) * 128].astype(BF16)) for uu in range(4)]
                    p0i = [x & tri_i32 for x in pmi]
                    acca = acca + pv_a(0, [_bf16_rows(x) for x in p0i])
                    acca = acca + pv_a(2, [_bf16_rows(x ^ y) for x, y in zip(pmi, p0i)])
                    normalize_store(ota, acca)
            if do_qk and c == CQA:
                qma = mask_q(qa[pl.ds(r1, 64), cs], j1)
                ss0, ss1 = [], []
                for uu in range(4):
                    us = slice(uu * 128, (uu + 1) * 128)
                    u = n * 4 + uu
                    if static_n and u == 0:
                        s3 = _dot(_bf16_rows(ka[g1, 128:192, :]), qma[:, us])
                        s1 = jnp.full((128, 128), NEG, F32)
                        sm = jnp.where(tri, NEG, s3)
                    elif static_n and u == 1:
                        s3 = _dot(_bf16_rows(ka[g1, 128:256, :]), qma[:, us])
                        s1 = s3[0:128]
                        sm = jnp.where(tri, NEG, s3[128:256])
                    else:
                        s3 = _dot(_bf16_rows(ka[g1, pl.ds(c02 + uu * 64, 192), :]), qma[:, us])
                        s1 = s3[128:256]
                        s0 = s3[0:128]
                        if not static_n:
                            s1 = jnp.where(u >= 1, s1, NEG)
                            s0 = jnp.where(u >= 2, s0, NEG)
                        sm = jnp.where(tri, s0, s3[256:384])
                    ss1.append(s1)
                    ss0.append(sm)
                s1 = jnp.concatenate(ss1, axis=1)
                sm = jnp.concatenate(ss0, axis=1)
                sa[0:128, cs] = s1
                sa[128:256, cs] = sm
                ma[:, cs] = jnp.max(jnp.maximum(s1, sm), axis=0, keepdims=True)
        if do_pv:
            normalize_store(otb, acc)
        if do_qk:
            mb[:, cs] = jnp.max(mx, axis=0, keepdims=True)

    def first_scores(n, carry):
        block(-1, n, True, False)
        return carry

    lax.fori_loop(0, S // NB, first_scores, 0)

    def head(h, gj):
        for n in range(S // NB):
            block(h, n, True, True, gj=gj)
        g1, j1 = gj
        wrap = j1 == HG - 1
        return jnp.where(wrap, g1 + 1, g1), jnp.where(wrap, 0, j1 + 1)

    lax.fori_loop(0, H - 1, head, (jnp.int32(0), jnp.int32(1)))

    for c in w_o:
        c.wait()

    def ocp(t):
        return pltpu.make_async_copy(
            obuf.at[t], out_hbm.at[pl.ds(pl.multiple_of(t * TC, TC), TC), :], osem.at[t])

    def outp(t, carry):
        ts = pl.ds(pl.multiple_of(t * TC, TC), TC)
        ys = [None, None]

        def hook(c):
            if c % 2 == 0:
                br, kt = divmod(c // 2, 4)
                ot, wo = ((ota, woa), (otb, wob))[br]
                rs = slice(kt * 128, (kt + 1) * 128)
                y = _dot_tn(wo[rs, :], ot[rs, ts].astype(BF16))
                ys[br] = y if ys[br] is None else ys[br] + y

        block(H - 1, t, False, True, hook)
        ya = ys[0] + _dot_tn(woa[512:, :], ota[512:, ts].astype(BF16))
        yb = ys[1] + _dot_tn(wob[512:, :], otb[512:, ts].astype(BF16))
        obuf[t] = jnp.concatenate([ya, yb], axis=0).astype(BF16).T
        ocp(t).start()
        return carry

    lax.fori_loop(0, NTC, outp, 0)
    for t in range(NTC):
        ocp(t).wait()


@jax.jit
def pallas_concat_heads__sliding_block__grouped_kv_mqa__prompt_kernel(
    A_x: jax.Array,
    A_wqkv: jax.Array,
    A_wo: jax.Array,
    B_x: jax.Array,
    B_wq: jax.Array,
    B_wk: jax.Array,
    B_wv: jax.Array,
    B_wo: jax.Array,
):
    hbm = pl.BlockSpec(memory_space=pl.ANY)
    out = pl.pallas_call(
        _kernel,
        out_shape=jax.ShapeDtypeStruct((S, 2 * D), BF16),
        in_specs=[hbm] * 8,
        out_specs=hbm,
        scratch_shapes=[
            pltpu.VMEM((D, S), BF16),
            pltpu.VMEM((D, S), BF16),
            pltpu.VMEM((D, 3 * D), BF16),
            pltpu.VMEM((D, D), BF16),
            pltpu.VMEM((D, D), BF16),
            pltpu.VMEM((D, D), BF16),
            pltpu.VMEM((DH, D), BF16),
            pltpu.VMEM((DH, D), BF16),
            pltpu.VMEM((NTC, TC, 2 * D), BF16),
            pltpu.SemaphoreType.DMA((6,)),
            pltpu.SemaphoreType.DMA((2 * NTC,)),
            pltpu.SemaphoreType.DMA((NTC,)),
            pltpu.VMEM((KVR, D), BF16),
            pltpu.VMEM((NG * 64, S), I32),
            pltpu.VMEM((NG, (S + PADK) // 2, 128), I32),
            pltpu.VMEM((D, S + PADK), F32),
            pltpu.VMEM((NG * 64, S), I32),
            pltpu.VMEM((S // 2, 128), I32),
            pltpu.VMEM((4, VR, S), F32),
            pltpu.VMEM((256, S), F32),
            pltpu.VMEM((S, S), F32),
            pltpu.VMEM((1, S), F32),
            pltpu.VMEM((1, S), F32),
            pltpu.VMEM((D, S), F32),
            pltpu.VMEM((D, S), F32),
        ],
        compiler_params=pltpu.CompilerParams(vmem_limit_bytes=120 * 1024 * 1024),
        name="fused_attn",
    )(A_x.reshape(S, D).T, A_wqkv, A_wo, B_x.reshape(S, D).T, B_wq, B_wk.T, B_wv.T, B_wo)
    return out.reshape(1, S, 2 * D)
```

```python
import math

import jax
import jax.numpy as jnp
from jax import lax
import jax.experimental.pallas as pl
import jax.experimental.pallas.tpu as pltpu

S = 2048
D = 576
H = 32
DH = 18
HG = 7
NG = 5
GW = HG * DH
NW = 4
CW = 128 // NW
HGA = (7 // NW) * NW
NGA = -(-H // HGA)
GWA = HGA * DH
VR = 24
PADK = 256
NB = 512
NCH = S // 128
TC = 512
NTC = S // TC
KVR = 48
CP1, CP0, CQA = 1, 4, 7
assert CP0 < 14
NEG = -1e30
SCALE = float(DH ** -0.5) * math.log2(math.e)
F32 = jnp.float32
BF16 = jnp.bfloat16
I32 = jnp.int32

TN = (((0,), (0,)), ((), ()))


def _dot(a, b):
    return jnp.dot(a, b, preferred_element_type=F32)


def _dot_tn(a, b):
    return lax.dot_general(a, b, TN, preferred_element_type=F32)


def _bf16_rows(x_i32):
    return pltpu.bitcast(x_i32, BF16)


def _pack_rows(x_bf16):
    return pltpu.bitcast(x_bf16, I32)


def _kernel(xa_hbm, wqkv_hbm, woa_hbm, xb_hbm, wq_hbm, wk_hbm, wv_hbm, wob_hbm, out_hbm,
            xa, xb, wqkv, woa, wob, wq, wk, wv, obuf, isem, xsem, osem,
            wkv, qa, ka, vta, qb, kb, vtb, sa, sb, ma, mb, ota, otb):
    def cp(i, src, dst):
        return pltpu.make_async_copy(src, dst, isem.at[i])

    def xcp(b, t):
        src, dst = ((xb_hbm, xb), (xa_hbm, xa))[b]
        ts = pl.ds(pl.multiple_of(t * TC, TC), TC)
        return pltpu.make_async_copy(src.at[:, ts], dst.at[:, ts], xsem.at[b * NTC + t])

    first = [cp(0, wk_hbm, wk), cp(1, wv_hbm, wv), cp(2, wq_hbm, wq)]
    w_a = cp(3, wqkv_hbm, wqkv)
    w_o = [cp(4, woa_hbm, woa), cp(5, wob_hbm, wob)]
    for c in first:
        c.start()
    xcp(0, 0).start()
    for g in range(NGA):
        ka[g, 0:PADK // 2, :] = jnp.zeros((PADK // 2, 128), I32)
    vta[:, 0:PADK] = jnp.zeros((D, PADK), F32)
    for c in first:
        c.wait()
    xcp(0, 1).start()
    xcp(0, 2).start()

    wkv[...] = jnp.concatenate(
        [wk[...].astype(F32), wv[...].astype(F32), jnp.zeros((KVR - 2 * DH, D), F32)],
        axis=0).astype(BF16)
    rowv = lax.broadcasted_iota(I32, (VR, TC), 0)

    def store_q(q_ref, rq, ts, ng, gw, last):
        for g in range(ng):
            gr = 128 if g < ng - 1 else last
            qf = rq[g * gw:min(g * gw + gr, rq.shape[0])]
            if qf.shape[0] < gr:
                qf = jnp.concatenate([qf, jnp.zeros((gr - qf.shape[0], TC), F32)], axis=0)
            q_ref[g * 64:g * 64 + gr // 2, ts] = _pack_rows((qf * SCALE).astype(BF16))

    def proj_b(t, carry):
        xcp(0, t).wait()

        @pl.when(t == 0)
        def _():
            xcp(0, 3).start()
            w_a.start()

        @pl.when(t == 1)
        def _():
            xcp(1, 0).start()
            for c in w_o:
                c.start()

        @pl.when(t == 2)
        def _():
            for u in range(1, NTC):
                xcp(1, u).start()

        ts = pl.ds(pl.multiple_of(t * TC, TC), TC)
        r = _dot(wkv[...], xb[:, ts])
        store_q(qb, _dot_tn(wq[...], xb[:, ts]), ts, NG, GW, 80)
        kt = r[0:DH]
        k16 = jnp.concatenate([kt] * HG + [kt[0:128 - GW]], axis=0).astype(BF16).T
        kb[pl.ds(pl.multiple_of(t * (TC // 2), TC // 2), TC // 2), :] = _pack_rows(k16)
        vt = r[DH:DH + VR].astype(BF16).astype(F32)
        vt = jnp.where(rowv == DH, 1.0, jnp.where(rowv < DH, vt, 0.0))
        for i in range(4):
            vtb[i, :, ts] = vt if i == 0 else pltpu.roll(vt, 2 * i, 0)
        return carry

    lax.fori_loop(0, NTC, proj_b, 0)

    w_a.wait()

    def proj_a(t, carry):
        xcp(1, t).wait()
        ts = pl.ds(pl.multiple_of(t * TC, TC), TC)
        tp = pl.ds(pl.multiple_of(PADK + t * TC, TC // 2), TC)
        tp2 = pl.ds(pl.multiple_of((PADK + t * TC) // 2, TC // 4), TC // 2)
        r = _dot_tn(wqkv[...], xa[:, ts])
        store_q(qa, r[0:2 * D], ts, NGA, GWA, 16 * -(-(D - (NGA - 1) * GWA) // 16))
        for g in range(NGA):
            ka[g, tp2, :] = _pack_rows(r[D + g * GWA:D + g * GWA + 128].astype(BF16).T)
        vta[:, tp] = r[2 * D:].astype(BF16).astype(F32)
        return carry

    lax.fori_loop(0, NTC, proj_a, 0)

    r64 = lax.broadcasted_iota(I32, (64, 128), 0)
    c64 = lax.broadcasted_iota(I32, (64, 128), 1)
    tri_i32 = jnp.where(2 * r64 > c64, 0xFFFF, 0) | jnp.where(2 * r64 + 1 > c64, -65536, 0)
    rvr = lax.broadcasted_iota(I32, (VR, 128), 0)
    c128 = lax.broadcasted_iota(I32, (128, 128), 1)
    rvr_b = lax.broadcasted_iota(I32, (VR, NB), 0)

    def mask_q(qi, j):
        row = lax.broadcasted_iota(I32, qi.shape, 0)
        return _bf16_rows(jnp.where((row >= (DH // 2) * j) & (row < (DH // 2) * (j + 1)), qi, 0))

    def block(h, n, do_qk, do_pv, hook=None, gj=None, ga1=(0, 0, 0), cp=(CP1, CP0)):
        static_n = isinstance(n, int)
        c0 = n * NB if static_n else pl.multiple_of(n * NB, NB)
        cs = pl.ds(c0, NB)
        if do_qk:
            g1, j1 = gj if gj is not None else divmod(h + 1, HG)
            r1 = g1 * 64 if isinstance(g1, int) else pl.multiple_of(g1 * 64, 64)
            qm = mask_q(qb[pl.ds(r1, 64), cs], j1)
        if do_pv:
            o = (h * DH) & 7
            w0 = h * DH - o
            w0 = w0 if isinstance(h, int) else pl.multiple_of(w0, 8)
            one_pos = jnp.where(o == 6, 0, o + DH) if not isinstance(h, int) else (o + DH) % VR
            vi = o >> 1
            m_cur = mb[:, cs]

        def normalize_store(dst, acc):
            l = jnp.sum(jnp.where(rvr_b == one_pos, acc, 0.0), axis=0, keepdims=True)
            pltpu.store(dst.at[pl.ds(w0, VR), cs], acc * (1.0 / l),
                        mask=(rvr_b >= o) & (rvr_b < o + DH))

        if do_pv:
            part = h % NW if isinstance(h, int) else h & (NW - 1)
            ha = h - part
            oa_ = [((ha + e) * DH) & 7 for e in range(NW)]
            wa_ = [(ha + e) * DH - oa_[e] for e in range(NW)]
            wa_ = [w if isinstance(w, int) else pl.multiple_of(w, 8) for w in wa_]
            onea = [(x + DH) % VR if isinstance(x, int) else jnp.where(x == 6, 0, x + DH) for x in oa_]
            ua = part * (16 // NW) + n * (4 // NW)
            OA = jnp.concatenate([jnp.full((VR, 128), x, I32) for _ in range(4 // NW) for x in oa_], axis=1)
            ONE = jnp.concatenate([jnp.full((VR, 128), x, I32) for _ in range(4 // NW) for x in onea], axis=1)

        def pv_a(t, pt):
            res = []
            for uu in range(4 // NW):
                col = pl.multiple_of((ua + uu + t) * 128, 128)
                for e in range(NW):
                    vt = vta[pl.ds(wa_[e], VR), pl.ds(col, 128)]
                    vt = jnp.where(rvr == onea[e], 1.0, vt)
                    res.append(_dot(vt, pt[NW * uu + e]))
            return jnp.concatenate(res, axis=1)

        def tiles(p):
            return [_pack_rows(p[:, i * 128:(i + 1) * 128].astype(BF16)) for i in range(4)]

        acc = mx = acca = None
        for c in range(NCH):
            ks = slice(c * 128, (c + 1) * 128)
            if hook is not None:
                hook(c)
            if do_pv:
                p = jnp.exp2(sb[ks, cs] - m_cur).astype(BF16)
                d = _dot(vtb[vi, :, ks], p)
                acc = d if acc is None else acc + d
            if do_qk:
                s = _dot(_bf16_rows(kb[c * 64:(c + 1) * 64, :]), qm)
                sb[ks, cs] = s
                mc = jnp.max(s.reshape(16, 8, NB), axis=0)
                mx = mc if mx is None else jnp.maximum(mx, mc)
            if do_pv:
                if c == cp[0]:
                    m_a = ma[:, cs]
                    p1 = tiles(jnp.exp2(sa[0:128, cs] - m_a))
                    acca = pv_a(1, [_bf16_rows(x) for x in p1])
                if c == cp[1]:
                    pmi = tiles(jnp.exp2(sa[128:256, cs] - m_a))
                    p0i = [x & tri_i32 for x in pmi]
                    acca = acca + pv_a(0, [_bf16_rows(x) for x in p0i])
                    acca = acca + pv_a(2, [_bf16_rows(x ^ y) for x, y in zip(pmi, p0i)])
                    l = jnp.sum(jnp.where(rvr_b == ONE, acca, 0.0), axis=0, keepdims=True)
                    on = acca * (1.0 / l)
                    msk = (rvr_b >= OA) & (rvr_b < OA + DH)
                    for uu in range(4 // NW):
                        col = pl.multiple_of((ua + uu) * 128, 128)
                        for e in range(NW):
                            ls = slice((NW * uu + e) * 128, (NW * uu + e + 1) * 128)
                            pltpu.store(ota.at[pl.ds(wa_[e], VR), pl.ds(col, 128)], on[:, ls], mask=msk[:, ls])
            if do_qk and c == CQA:
                ga, ja, part1 = ga1
                ra = ga * 64 if isinstance(ga, int) else pl.multiple_of(ga * 64, 64)
                mk = [(r64 >= (DH // 2) * (ja + e)) & (r64 < (DH // 2) * (ja + e + 1)) for e in range(NW)]
                seg64 = [(c64 >= e * CW) & (c64 < (e + 1) * CW) for e in range(NW)]
                seg128 = [(c128 >= e * CW) & (c128 < (e + 1) * CW) for e in range(NW)]
                tri_cw = (lax.broadcasted_iota(I32, (CW, 128), 0)
                          > (lax.broadcasted_iota(I32, (CW, 128), 1) & (CW - 1)))

                def rolled(x, sh):
                    return x if sh % 128 == 0 else pltpu.roll(x, sh % 128, 1)

                def pick(segs, parts):
                    out = parts[-1]
                    for e in range(len(parts) - 2, -1, -1):
                        out = jnp.where(segs[e], parts[e], out)
                    return out

                ss0, ss1 = [], []
                for uu in range(4 // NW):
                    u = part1 * (16 // NW) + n * (4 // NW) + uu
                    q0 = qa[pl.ds(ra, 64), pl.ds(pl.multiple_of(u * 128, 128), 128)]
                    qr = [rolled(q0, i * CW) for i in range(NW)]
                    ys, zs = [], []
                    for k in range(NW):
                        wk_ = pick(seg64, [jnp.where(mk[e], qr[(e - k) % NW], 0) for e in range(NW)])
                        k0 = pl.multiple_of(u * 64 + k * (CW // 2), CW // 2)
                        x = _dot(_bf16_rows(ka[ga, pl.ds(k0, (256 + CW) // 2), :]), _bf16_rows(wk_))
                        n0 = 128 - k * CW
                        t0, z, t2 = x[0:n0], x[n0:n0 + 128], x[n0 + 128:]
                        if (not static_n) or n * (4 // NW) + uu < 2:
                            t0 = jnp.where(u >= 2, t0, NEG)
                            z = jnp.where(u >= 1, z, NEG)
                        y = [jnp.where(tri_cw, t0[0:CW], t2[k * CW:])]
                        if k > 0:
                            y = [t2[0:k * CW]] + y
                        if k < NW - 1:
                            y = y + [t0[CW:]]
                        ys.append(jnp.concatenate(y, axis=0))
                        zs.append(z)
                    for e in range(NW):
                        ss1.append(pick(seg128, [rolled(zs[k], (k - e) * CW) for k in range(NW)]))
                        ss0.append(pick(seg128, [rolled(ys[k], (k - e) * CW) for k in range(NW)]))
                s1 = jnp.concatenate(ss1, axis=1)
                sm = jnp.concatenate(ss0, axis=1)
                sa[0:128, cs] = s1
                sa[128:256, cs] = sm
                ma[:, cs] = jnp.max(jnp.maximum(s1, sm), axis=0, keepdims=True)
        if do_pv:
            normalize_store(otb, acc)
        if do_qk:
            mb[:, cs] = jnp.max(mx, axis=0, keepdims=True)

    def first_scores(n, carry):
        block(-1, n, True, False)
        return carry

    lax.fori_loop(0, S // NB, first_scores, 0)

    def head(h, st):
        g1, j1, ga, ja = st
        part1 = (h + 1) & (NW - 1)
        for n in range(S // NB):
            block(h, n, True, True, gj=(g1, j1), ga1=(ga, ja, part1))
        wrap = j1 == HG - 1
        adv = part1 == NW - 1
        wrapa = adv & (ja == HGA - NW)
        return (jnp.where(wrap, g1 + 1, g1), jnp.where(wrap, 0, j1 + 1),
                jnp.where(wrapa, ga + 1, ga), jnp.where(wrapa, 0, jnp.where(adv, ja + NW, ja)))

    lax.fori_loop(0, H - 1, head, (jnp.int32(0), jnp.int32(1), jnp.int32(0), jnp.int32(0)))

    for c in w_o:
        c.wait()

    def ocp(t):
        return pltpu.make_async_copy(
            obuf.at[t], out_hbm.at[pl.ds(pl.multiple_of(t * TC, TC), TC), :], osem.at[t])

    def outp(t, carry):
        ts = pl.ds(pl.multiple_of(t * TC, TC), TC)
        ys = [None, None]

        def hook(c):
            if c % 2 == 0:
                br, kt = divmod(c // 2 + 4, 8)[1] // 4, (c // 2) % 4
                ot, wo = ((ota, woa), (otb, wob))[br]
                rs = slice(kt * 128, (kt + 1) * 128)
                y = _dot_tn(wo[rs, :], ot[rs, ts].astype(BF16))
                ys[br] = y if ys[br] is None else ys[br] + y

        block(H - 1, t, False, True, hook, cp=(1, 4))
        ya = ys[0] + _dot_tn(woa[512:, :], ota[512:, ts].astype(BF16))
        yb = ys[1] + _dot_tn(wob[512:, :], otb[512:, ts].astype(BF16))
        obuf[t] = jnp.concatenate([ya, yb], axis=0).astype(BF16).T
        ocp(t).start()
        return carry

    lax.fori_loop(0, NTC, outp, 0)
    for t in range(NTC):
        ocp(t).wait()


@jax.jit
def pallas_concat_heads__sliding_block__grouped_kv_mqa__prompt_kernel(
    A_x: jax.Array,
    A_wqkv: jax.Array,
    A_wo: jax.Array,
    B_x: jax.Array,
    B_wq: jax.Array,
    B_wk: jax.Array,
    B_wv: jax.Array,
    B_wo: jax.Array,
):
    hbm = pl.BlockSpec(memory_space=pl.ANY)
    out = pl.pallas_call(
        _kernel,
        out_shape=jax.ShapeDtypeStruct((S, 2 * D), BF16),
        in_specs=[hbm] * 8,
        out_specs=hbm,
        scratch_shapes=[
            pltpu.VMEM((D, S), BF16),
            pltpu.VMEM((D, S), BF16),
            pltpu.VMEM((D, 3 * D), BF16),
            pltpu.VMEM((D, D), BF16),
            pltpu.VMEM((D, D), BF16),
            pltpu.VMEM((D, D), BF16),
            pltpu.VMEM((DH, D), BF16),
            pltpu.VMEM((DH, D), BF16),
            pltpu.VMEM((NTC, TC, 2 * D), BF16),
            pltpu.SemaphoreType.DMA((6,)),
            pltpu.SemaphoreType.DMA((2 * NTC,)),
            pltpu.SemaphoreType.DMA((NTC,)),
            pltpu.VMEM((KVR, D), BF16),
            pltpu.VMEM((NGA * 64, S), I32),
            pltpu.VMEM((NGA, (S + PADK) // 2, 128), I32),
            pltpu.VMEM((D, S + PADK), F32),
            pltpu.VMEM((NG * 64, S), I32),
            pltpu.VMEM((S // 2, 128), I32),
            pltpu.VMEM((4, VR, S), F32),
            pltpu.VMEM((256, S), F32),
            pltpu.VMEM((S, S), F32),
            pltpu.VMEM((1, S), F32),
            pltpu.VMEM((1, S), F32),
            pltpu.VMEM((D, S), F32),
            pltpu.VMEM((D, S), F32),
        ],
        compiler_params=pltpu.CompilerParams(vmem_limit_bytes=120 * 1024 * 1024),
        name="fused_attn",
    )(A_x.reshape(S, D).T, A_wqkv, A_wo, B_x.reshape(S, D).T, B_wq, B_wk.T, B_wv.T, B_wo)
    return out.reshape(1, S, 2 * D)
```

```python
import math

import jax
import jax.numpy as jnp
from jax import lax
import jax.experimental.pallas as pl
import jax.experimental.pallas.tpu as pltpu

S = 2048
D = 576
H = 32
DH = 18
HG = 7
NG = 5
GW = HG * DH
NW = 4
CW = 128 // NW
HGA = (7 // NW) * NW
NGA = -(-H // HGA)
GWA = HGA * DH
VR = 24
PADK = 256
NB = 512
NCH = S // 128
TC = 512
NTC = S // TC
KVR = 48
CP1, CP0, CQA = 2, 4, 7
assert CP0 < 14
NEG = -1e30
SCALE = float(DH ** -0.5) * math.log2(math.e)
F32 = jnp.float32
BF16 = jnp.bfloat16
I32 = jnp.int32

TN = (((0,), (0,)), ((), ()))


def _dot(a, b):
    return jnp.dot(a, b, preferred_element_type=F32)


def _dot_tn(a, b):
    return lax.dot_general(a, b, TN, preferred_element_type=F32)


def _bf16_rows(x_i32):
    return pltpu.bitcast(x_i32, BF16)


def _pack_rows(x_bf16):
    return pltpu.bitcast(x_bf16, I32)


def _kernel(xa_hbm, wqkv_hbm, woa_hbm, xb_hbm, wq_hbm, wk_hbm, wv_hbm, wob_hbm, out_hbm,
            xa, xb, wqkv, woa, wob, wq, wk, wv, obuf, isem, xsem, osem,
            wkv, qa, ka, vta, qb, kb, vtb, sa, sb, ma, mb, ota, otb):
    def cp(i, src, dst):
        return pltpu.make_async_copy(src, dst, isem.at[i])

    def xcp(b, t):
        src, dst = ((xb_hbm, xb), (xa_hbm, xa))[b]
        ts = pl.ds(pl.multiple_of(t * TC, TC), TC)
        return pltpu.make_async_copy(src.at[:, ts], dst.at[:, ts], xsem.at[b * NTC + t])

    first = [cp(0, wk_hbm, wk), cp(1, wv_hbm, wv), cp(2, wq_hbm, wq)]
    w_a = cp(3, wqkv_hbm, wqkv)
    w_o = [cp(4, woa_hbm, woa), cp(5, wob_hbm, wob)]
    for c in first:
        c.start()
    xcp(0, 0).start()
    for g in range(NGA):
        ka[g, 0:PADK // 2, :] = jnp.zeros((PADK // 2, 128), I32)
    vta[:, 0:PADK] = jnp.zeros((D, PADK), F32)
    qa[(NGA - 1) * 64 + 40:, :] = jnp.zeros((24, S), I32)
    qb[(NG - 1) * 64 + 40:, :] = jnp.zeros((24, S), I32)
    for c in first:
        c.wait()
    xcp(0, 1).start()
    xcp(0, 2).start()

    wkv[...] = jnp.concatenate(
        [wk[...].astype(F32), wv[...].astype(F32), jnp.zeros((KVR - 2 * DH, D), F32)],
        axis=0).astype(BF16)
    rowv = lax.broadcasted_iota(I32, (VR, TC), 0)

    def store_q(q_ref, rq, ts, ng, gw, last):
        for g in range(ng):
            gr = 128 if g < ng - 1 else last
            qf = rq[g * gw:min(g * gw + gr, rq.shape[0])]
            if qf.shape[0] < gr:
                qf = jnp.concatenate([qf, jnp.zeros((gr - qf.shape[0], TC), F32)], axis=0)
            q_ref[g * 64:g * 64 + gr // 2, ts] = _pack_rows((qf * SCALE).astype(BF16))

    def proj_b(t, carry):
        xcp(0, t).wait()

        @pl.when(t == 0)
        def _():
            xcp(0, 3).start()
            w_a.start()

        @pl.when(t == 1)
        def _():
            xcp(1, 0).start()
            for c in w_o:
                c.start()

        @pl.when(t == 2)
        def _():
            for u in range(1, NTC):
                xcp(1, u).start()

        ts = pl.ds(pl.multiple_of(t * TC, TC), TC)
        r = _dot(wkv[...], xb[:, ts])
        store_q(qb, _dot_tn(wq[...], xb[:, ts]), ts, NG, GW, 80)
        kt = r[0:DH]
        k16 = jnp.concatenate([kt] * HG + [kt[0:128 - GW]], axis=0).astype(BF16).T
        kb[pl.ds(pl.multiple_of(t * (TC // 2), TC // 2), TC // 2), :] = _pack_rows(k16)
        vt = r[DH:DH + VR].astype(BF16).astype(F32)
        vt = jnp.where(rowv == DH, 1.0, jnp.where(rowv < DH, vt, 0.0))
        for i in range(4):
            vtb[i, :, ts] = vt if i == 0 else pltpu.roll(vt, 2 * i, 0)
        return carry

    lax.fori_loop(0, NTC, proj_b, 0)

    w_a.wait()

    def proj_a(t, carry):
        xcp(1, t).wait()
        ts = pl.ds(pl.multiple_of(t * TC, TC), TC)
        tp = pl.ds(pl.multiple_of(PADK + t * TC, TC // 2), TC)
        tp2 = pl.ds(pl.multiple_of((PADK + t * TC) // 2, TC // 4), TC // 2)
        r = _dot_tn(wqkv[...], xa[:, ts])
        store_q(qa, r[0:2 * D], ts, NGA, GWA, 16 * -(-(D - (NGA - 1) * GWA) // 16))
        for g in range(NGA):
            ka[g, tp2, :] = _pack_rows(r[D + g * GWA:D + g * GWA + 128].astype(BF16).T)
        vta[:, tp] = r[2 * D:].astype(BF16).astype(F32)
        return carry

    lax.fori_loop(0, NTC, proj_a, 0)

    r64 = lax.broadcasted_iota(I32, (64, 128), 0)
    c64 = lax.broadcasted_iota(I32, (64, 128), 1)
    tri_i32 = jnp.where(2 * r64 > c64, 0xFFFF, 0) | jnp.where(2 * r64 + 1 > c64, -65536, 0)
    rvr = lax.broadcasted_iota(I32, (VR, 128), 0)
    c128 = lax.broadcasted_iota(I32, (128, 128), 1)
    rvr_b = lax.broadcasted_iota(I32, (VR, NB), 0)

    def mask_q(qi, j):
        row = lax.broadcasted_iota(I32, qi.shape, 0)
        return _bf16_rows(jnp.where((row >= (DH // 2) * j) & (row < (DH // 2) * (j + 1)), qi, 0))

    def block(h, n, do_qk, do_pv, hook=None, gj=None, ga1=(0, 0, 0), cp=(CP1, CP0)):
        static_n = isinstance(n, int)
        c0 = n * NB if static_n else pl.multiple_of(n * NB, NB)
        cs = pl.ds(c0, NB)
        if do_qk:
            g1, j1 = gj if gj is not None else divmod(h + 1, HG)
            r1 = g1 * 64 if isinstance(g1, int) else pl.multiple_of(g1 * 64, 64)
            qm = mask_q(qb[pl.ds(r1, 64), cs], j1)
        if do_pv:
            o = (h * DH) & 7
            w0 = h * DH - o
            w0 = w0 if isinstance(h, int) else pl.multiple_of(w0, 8)
            one_pos = jnp.where(o == 6, 0, o + DH) if not isinstance(h, int) else (o + DH) % VR
            vi = o >> 1
            m_cur = mb[:, cs]

        def normalize_store(dst, acc):
            l = jnp.sum(jnp.where(rvr_b == one_pos, acc, 0.0), axis=0, keepdims=True)
            pltpu.store(dst.at[pl.ds(w0, VR), cs], acc * (1.0 / l),
                        mask=(rvr_b >= o) & (rvr_b < o + DH))

        if do_pv:
            part = h % NW if isinstance(h, int) else h & (NW - 1)
            ha = h - part
            oa_ = [((ha + e) * DH) & 7 for e in range(NW)]
            wa_ = [(ha + e) * DH - oa_[e] for e in range(NW)]
            wa_ = [w if isinstance(w, int) else pl.multiple_of(w, 8) for w in wa_]
            onea = [(x + DH) % VR if isinstance(x, int) else jnp.where(x == 6, 0, x + DH) for x in oa_]
            ua = part * (16 // NW) + n * (4 // NW)
            OA = jnp.concatenate([jnp.full((VR, 128), x, I32) for _ in range(4 // NW) for x in oa_], axis=1)
            ONE = jnp.concatenate([jnp.full((VR, 128), x, I32) for _ in range(4 // NW) for x in onea], axis=1)

        def pv_a(t, pt):
            res = []
            for uu in range(4 // NW):
                col = pl.multiple_of((ua + uu + t) * 128, 128)
                for e in range(NW):
                    vt = vta[pl.ds(wa_[e], VR), pl.ds(col, 128)]
                    vt = jnp.where(rvr == onea[e], 1.0, vt)
                    res.append(_dot(vt, pt[NW * uu + e]))
            return jnp.concatenate(res, axis=1)

        def tiles(p):
            return [_pack_rows(p[:, i * 128:(i + 1) * 128].astype(BF16)) for i in range(4)]

        acc = mx = acca = None
        for c in range(NCH):
            ks = slice(c * 128, (c + 1) * 128)
            if hook is not None:
                hook(c)
            if do_pv:
                p = jnp.exp2(sb[ks, cs] - m_cur).astype(BF16)
                d = _dot(vtb[vi, :, ks], p)
                acc = d if acc is None else acc + d
            if do_qk:
                s = _dot(_bf16_rows(kb[c * 64:(c + 1) * 64, :]), qm)
                sb[ks, cs] = s
                mc = jnp.max(s.reshape(16, 8, NB), axis=0)
                mx = mc if mx is None else jnp.maximum(mx, mc)
            if do_pv:
                if c == cp[0]:
                    m_a = ma[:, cs]
                    p1 = tiles(jnp.exp2(sa[0:128, cs] - m_a))
                    acca = pv_a(1, [_bf16_rows(x) for x in p1])
                if c == cp[1]:
                    pmi = tiles(jnp.exp2(sa[128:256, cs] - m_a))
                    p0i = [x & tri_i32 for x in pmi]
                    acca = acca + pv_a(0, [_bf16_rows(x) for x in p0i])
                    acca = acca + pv_a(2, [_bf16_rows(x ^ y) for x, y in zip(pmi, p0i)])
                    l = jnp.sum(jnp.where(rvr_b == ONE, acca, 0.0), axis=0, keepdims=True)
                    on = acca * (1.0 / l)
                    msk = (rvr_b >= OA) & (rvr_b < OA + DH)
                    for uu in range(4 // NW):
                        col = pl.multiple_of((ua + uu) * 128, 128)
                        for e in range(NW):
                            ls = slice((NW * uu + e) * 128, (NW * uu + e + 1) * 128)
                            pltpu.store(ota.at[pl.ds(wa_[e], VR), pl.ds(col, 128)], on[:, ls], mask=msk[:, ls])
            if do_qk and c == CQA:
                ga, ja, part1 = ga1
                ra = ga * 64 if isinstance(ga, int) else pl.multiple_of(ga * 64, 64)
                mk = [(r64 >= (DH // 2) * (ja + e)) & (r64 < (DH // 2) * (ja + e + 1)) for e in range(NW)]
                seg64 = [(c64 >= e * CW) & (c64 < (e + 1) * CW) for e in range(NW)]
                seg128 = [(c128 >= e * CW) & (c128 < (e + 1) * CW) for e in range(NW)]
                tri_cw = (lax.broadcasted_iota(I32, (CW, 128), 0)
                          > (lax.broadcasted_iota(I32, (CW, 128), 1) & (CW - 1)))

                def rolled(x, sh):
                    return x if sh % 128 == 0 else pltpu.roll(x, sh % 128, 1)

                def pick(segs, parts):
                    out = parts[-1]
                    for e in range(len(parts) - 2, -1, -1):
                        out = jnp.where(segs[e], parts[e], out)
                    return out

                ss0, ss1 = [], []
                for uu in range(4 // NW):
                    u = part1 * (16 // NW) + n * (4 // NW) + uu
                    q0 = qa[pl.ds(ra, 64), pl.ds(pl.multiple_of(u * 128, 128), 128)]
                    qr = [rolled(q0, i * CW) for i in range(NW)]
                    ys, zs = [], []
                    for k in range(NW):
                        wk_ = pick(seg64, [jnp.where(mk[e], qr[(e - k) % NW], 0) for e in range(NW)])
                        k0 = pl.multiple_of(u * 64 + k * (CW // 2), CW // 2)
                        x = _dot(_bf16_rows(ka[ga, pl.ds(k0, (256 + CW) // 2), :]), _bf16_rows(wk_))
                        n0 = 128 - k * CW
                        t0, z, t2 = x[0:n0], x[n0:n0 + 128], x[n0 + 128:]
                        if (not static_n) or n * (4 // NW) + uu < 2:
                            t0 = jnp.where(u >= 2, t0, NEG)
                            z = jnp.where(u >= 1, z, NEG)
                        y = [jnp.where(tri_cw, t0[0:CW], t2[k * CW:])]
                        if k > 0:
                            y = [t2[0:k * CW]] + y
                        if k < NW - 1:
                            y = y + [t0[CW:]]
                        ys.append(jnp.concatenate(y, axis=0))
                        zs.append(z)
                    for e in range(NW):
                        ss1.append(pick(seg128, [rolled(zs[k], (k - e) * CW) for k in range(NW)]))
                        ss0.append(pick(seg128, [rolled(ys[k], (k - e) * CW) for k in range(NW)]))
                s1 = jnp.concatenate(ss1, axis=1)
                sm = jnp.concatenate(ss0, axis=1)
                sa[0:128, cs] = s1
                sa[128:256, cs] = sm
                ma[:, cs] = jnp.max(jnp.maximum(s1, sm), axis=0, keepdims=True)
        if do_pv:
            normalize_store(otb, acc)
        if do_qk:
            mb[:, cs] = jnp.max(mx, axis=0, keepdims=True)

    def first_scores(n, carry):
        block(-1, n, True, False)
        return carry

    lax.fori_loop(0, S // NB, first_scores, 0)

    def head(h, st):
        g1, j1, ga, ja = st
        part1 = (h + 1) & (NW - 1)
        for n in range(S // NB):
            block(h, n, True, True, gj=(g1, j1), ga1=(ga, ja, part1))
        wrap = j1 == HG - 1
        adv = part1 == NW - 1
        wrapa = adv & (ja == HGA - NW)
        return (jnp.where(wrap, g1 + 1, g1), jnp.where(wrap, 0, j1 + 1),
                jnp.where(wrapa, ga + 1, ga), jnp.where(wrapa, 0, jnp.where(adv, ja + NW, ja)))

    lax.fori_loop(0, H - 1, head, (jnp.int32(0), jnp.int32(1), jnp.int32(0), jnp.int32(0)))

    for c in w_o:
        c.wait()

    def ocp(t):
        return pltpu.make_async_copy(
            obuf.at[t], out_hbm.at[pl.ds(pl.multiple_of(t * TC, TC), TC), :], osem.at[t])

    def outp(t, carry):
        ts = pl.ds(pl.multiple_of(t * TC, TC), TC)
        ys = [None, None]

        def hook(c):
            if c % 2 == 0:
                br, kt = divmod(c // 2 + 4, 8)[1] // 4, (c // 2) % 4
                ot, wo = ((ota, woa), (otb, wob))[br]
                rs = slice(kt * 128, (kt + 1) * 128)
                y = _dot_tn(wo[rs, :], ot[rs, ts].astype(BF16))
                ys[br] = y if ys[br] is None else ys[br] + y

        block(H - 1, t, False, True, hook, cp=(CP1, CP0))
        ya = ys[0] + _dot_tn(woa[512:, :], ota[512:, ts].astype(BF16))
        yb = ys[1] + _dot_tn(wob[512:, :], otb[512:, ts].astype(BF16))
        obuf[t] = jnp.concatenate([ya, yb], axis=0).astype(BF16).T
        ocp(t).start()
        return carry

    lax.fori_loop(0, NTC, outp, 0)
    for t in range(NTC):
        ocp(t).wait()


@jax.jit
def pallas_concat_heads__sliding_block__grouped_kv_mqa__prompt_kernel(
    A_x: jax.Array,
    A_wqkv: jax.Array,
    A_wo: jax.Array,
    B_x: jax.Array,
    B_wq: jax.Array,
    B_wk: jax.Array,
    B_wv: jax.Array,
    B_wo: jax.Array,
):
    hbm = pl.BlockSpec(memory_space=pl.ANY)
    out = pl.pallas_call(
        _kernel,
        out_shape=jax.ShapeDtypeStruct((S, 2 * D), BF16),
        in_specs=[hbm] * 8,
        out_specs=hbm,
        scratch_shapes=[
            pltpu.VMEM((D, S), BF16),
            pltpu.VMEM((D, S), BF16),
            pltpu.VMEM((D, 3 * D), BF16),
            pltpu.VMEM((D, D), BF16),
            pltpu.VMEM((D, D), BF16),
            pltpu.VMEM((D, D), BF16),
            pltpu.VMEM((DH, D), BF16),
            pltpu.VMEM((DH, D), BF16),
            pltpu.VMEM((NTC, TC, 2 * D), BF16),
            pltpu.SemaphoreType.DMA((6,)),
            pltpu.SemaphoreType.DMA((2 * NTC,)),
            pltpu.SemaphoreType.DMA((NTC,)),
            pltpu.VMEM((KVR, D), BF16),
            pltpu.VMEM((NGA * 64, S), I32),
            pltpu.VMEM((NGA, (S + PADK) // 2, 128), I32),
            pltpu.VMEM((D, S + PADK), F32),
            pltpu.VMEM((NG * 64, S), I32),
            pltpu.VMEM((S // 2, 128), I32),
            pltpu.VMEM((4, VR, S), F32),
            pltpu.VMEM((256, S), F32),
            pltpu.VMEM((S, S), F32),
            pltpu.VMEM((1, S), F32),
            pltpu.VMEM((1, S), F32),
            pltpu.VMEM((D, S), F32),
            pltpu.VMEM((D, S), F32),
        ],
        compiler_params=pltpu.CompilerParams(
            vmem_limit_bytes=120 * 1024 * 1024,
            flags={"XLA_TPU_EVENLY_DISTRIBUTE_CRITICAL_NODES": True}),
        name="fused_attn",
    )(A_x.reshape(S, D).T, A_wqkv, A_wo, B_x.reshape(S, D).T, B_wq, B_wk.T, B_wv.T, B_wo)
    return out.reshape(1, S, 2 * D)
```
